```python
import jax
import jax.numpy as jnp

def _softmax(x, axis=-1):
    return jax.nn.softmax(x, axis=axis)
def _gelu(x):
    return jax.nn.gelu(x, approximate=True)
def _silu(x):
    return jax.nn.silu(x)
def _sigmoid(x):
    return jax.nn.sigmoid(x)
def _layernorm(x, axis=-1, eps=1e-5):
    m = jnp.mean(x, axis=axis, keepdims=True)
    v = jnp.var(x, axis=axis, keepdims=True)
    return (x - m) / jnp.sqrt(v + eps)
def _scatter_add(tgt, idx, src, axis=0):
    return tgt.at[idx].add(src)
def _segment_sum(src, seg, n):
    return jax.ops.segment_sum(src, seg, n)
class _Rng:
    def __init__(self, key):
        self._k = key
    def _next(self):
        self._k, sub = jax.random.split(self._k)
        return sub
    def normal(self, shape):
        return jax.random.normal(self._next(), shape, dtype=jnp.bfloat16)
    def randint(self, lo, hi, shape):
        return jax.random.randint(self._next(), shape, lo, hi, dtype=jnp.int32)
    def uniform(self, shape, lo=0.0, hi=1.0):
        return jax.random.uniform(self._next(), shape, jnp.bfloat16, lo, hi)
    def permutation(self, n):
        return jax.random.permutation(self._next(), n)


kernel_name = 'gated_mix__mha_block_cached__moe_arch_mod__decode'

def setup_inputs():
    _rng = _Rng(jax.random.key(int.from_bytes(__import__("os").urandom(4), "little")))
    _w = (lambda a: (lambda t: t.astype(jnp.bfloat16) if jnp.issubdtype(t.dtype, jnp.floating) else t)(jnp.asarray(a)))
    def _A_setup():
        B, Sq, D = 4, 1, 1024
        H, Sk, Dh = 32, 8192, 128
        return {
            "x": _w((lambda *s: _rng.normal(s) * 0.05)(B, Sq, D)),
            "k_cache": _w((lambda *s: _rng.normal(s) * 0.05)(B, H, Sk, Dh)),
            "v_cache": _w((lambda *s: _rng.normal(s) * 0.05)(B, H, Sk, Dh)),
            "wq": _w((lambda *s: _rng.normal(s) * 0.05)(D, H * Dh) * (D ** -0.5)),
            "wo": _w((lambda *s: _rng.normal(s) * 0.05)(H * Dh, D) * ((H * Dh) ** -0.5)),
        }
    _A_in = _A_setup()

    def _B_setup():
        B, S, D, F, C = 4, 1, 1024, 3584, 1
        return {
            "x": _w((lambda *s: _rng.normal(s) * 0.05)(B, S, D)),
            "w_r": _w((lambda *s: _rng.normal(s) * 0.05)(D)),
            "w_gate": _w((lambda *s: _rng.normal(s) * 0.05)(D, F)),
            "w_up": _w((lambda *s: _rng.normal(s) * 0.05)(D, F)),
            "w_down": _w((lambda *s: _rng.normal(s) * 0.05)(F, D)),
        }
    _B_in = _B_setup()

    return {
        "A_x": _A_in["x"],
        "A_k_cache": _A_in["k_cache"],
        "A_v_cache": _A_in["v_cache"],
        "A_wq": _A_in["wq"],
        "A_wo": _A_in["wo"],
        "B_x": _B_in["x"],
        "B_w_r": _B_in["w_r"],
        "B_w_gate": _B_in["w_gate"],
        "B_w_up": _B_in["w_up"],
        "B_w_down": _B_in["w_down"],
        "gate_w": _w((lambda *s: _rng.normal(s) * 0.05)(1024)),
    }

def reference(A_x, A_k_cache, A_v_cache, A_wq, A_wo, B_x, B_w_r, B_w_gate, B_w_up, B_w_down, gate_w):
    def _A_ref(x, k_cache, v_cache, wq, wo):
        B, Sq, D = x.shape
        H, Dh = 32, 128
        q = (lambda x, *d: x.transpose(*d))((x @ wq).reshape(B, Sq, H, Dh), 0, 2, 1, 3)
        scores = jnp.einsum("bhqd,bhkd->bhqk", q, k_cache) * (Dh ** -0.5)
        p = _softmax(scores, axis=-1)
        o = jnp.einsum("bhqk,bhkd->bhqd", p, v_cache)
        return (lambda x, *d: x.transpose(*d))(o, 0, 2, 1, 3).reshape(B, Sq, H * Dh) @ wo

    def _B_ref(x, w_r, w_gate, w_up, w_down):
        B, S, D = x.shape
        C = 1
        r = x @ w_r
        idx = jnp.argsort(-r, axis=-1)[:, :C]
        idx_e = jnp.repeat(idx.reshape(B, C, 1), D, axis=2)
        x_sel = jnp.take_along_axis(x, idx_e, axis=1)
        g = _silu(x_sel @ w_gate)
        u = x_sel @ w_up
        y = (g * u) @ w_down
        r_sel = _sigmoid(jnp.take_along_axis(r, idx, axis=1))
        y = y * r_sel.reshape(B, C, 1)
        b_off = (jnp.arange(B) * S).reshape(B, 1)
        flat_idx = (idx + b_off).reshape(B * C)
        zero = (x * 0.0).reshape(B * S, D)
        upd = _scatter_add(zero, flat_idx, y.reshape(B * C, D), axis=0)
        return x + upd.reshape(B, S, D)

    x = A_x
    g = _sigmoid((x * gate_w).sum(-1, keepdims=True))
    a = _A_ref(x, A_k_cache, A_v_cache, A_wq, A_wo)
    b = _B_ref(x, B_w_r, B_w_gate, B_w_up, B_w_down)
    return g * a + (1 - g) * b
```

```python
import functools

import jax
import jax.numpy as jnp
import jax.experimental.pallas as pl
import jax.experimental.pallas.tpu as pltpu

_NBUF = 4
_KV_ROWS = 128
_W_ROWS = 16
_W_COLS = 1024
_F32 = jnp.float32
_BF16 = jnp.bfloat16


def _start_weight(w_hbm, w_vmem, sem):
    rows, cols = w_hbm.shape
    col_starts = list(range(0, cols, _W_COLS))
    group = 2 * _W_ROWS

    def body(i, carry):
        for half in range(2):
            r0 = pl.multiple_of(i * group + half * _W_ROWS, _W_ROWS)
            for c0 in col_starts:
                cw = min(_W_COLS, cols - c0)
                pltpu.make_async_copy(
                    w_hbm.at[pl.ds(r0, _W_ROWS), pl.ds(c0, cw)],
                    w_vmem.at[pl.ds(r0, _W_ROWS), pl.ds(c0, cw)],
                    sem,
                ).start(priority=half)
        return carry

    jax.lax.fori_loop(0, rows // group, body, 0)


def _wait_all(buf, sem):
    pltpu.make_async_copy(buf, buf, sem).wait()


def _as_row(w_ref):
    w = w_ref[...].astype(_F32)
    return jnp.concatenate([w[j:j + 1, :] for j in range(w.shape[0])], axis=1)


def _kernel(ax_hbm, k_hbm, v_hbm, wq_hbm, wo_hbm, bx_hbm, wr_hbm, wg_hbm, wu_hbm,
            wd_hbm, gw_hbm, out_ref,
            ax_v, bx_v, wr_v, gw_v, wq_v, wo_v, wg_v, wu_v, wd_v, kbuf, vbuf,
            x_s, q_s, h_s, b_s, g_s, acc_s, ksem, vsem, wsem, ssem):
    nb, nh, sk, dh = k_hbm.shape
    nstep = nb * nh
    scale = dh ** -0.5

    def start_cache(src, buf, sem, step, priority):
        b = step % nb
        h = step // nb
        slot = step % _NBUF
        for j in range(sk // _KV_ROWS):
            rows = pl.ds(j * _KV_ROWS, _KV_ROWS)
            pltpu.make_async_copy(
                src.at[b, h, rows], buf.at[slot, rows], sem.at[slot]
            ).start(priority=priority)

    def start_kv(step):
        start_cache(k_hbm, kbuf, ksem, step, 0)
        start_cache(v_hbm, vbuf, vsem, step, 1)

    small = [
        pltpu.make_async_copy(ax_hbm, ax_v, ssem.at[0]),
        pltpu.make_async_copy(bx_hbm, bx_v, ssem.at[1]),
        pltpu.make_async_copy(wr_hbm, wr_v, ssem.at[2]),
        pltpu.make_async_copy(gw_hbm, gw_v, ssem.at[3]),
    ]
    for c in small:
        c.start()
    _start_weight(wq_hbm, wq_v, wsem.at[0])

    def prologue_kv(step, carry):
        start_kv(step)
        return carry

    jax.lax.fori_loop(0, _NBUF, prologue_kv, 0)
    _start_weight(wo_hbm, wo_v, wsem.at[1])
    for c in small:
        c.wait()

    x_s[...] = jnp.zeros(x_s.shape, _F32)
    x_s[0, pl.ds(0, nb), :] = ax_v[...].astype(_F32)
    x_s[1, pl.ds(0, nb), :] = bx_v[...].astype(_F32)
    ax = x_s[0]
    gate_w = _as_row(gw_v)
    g_s[...] = jax.nn.sigmoid(jnp.sum(ax * gate_w, axis=-1, keepdims=True))
    acc_s[...] = jnp.zeros(acc_s.shape, _F32)

    _wait_all(wq_v, wsem.at[0])
    ax_bf = ax.astype(_BF16)
    for h in range(nh):
        q_s[h] = jnp.dot(ax_bf, wq_v[:, pl.ds(h * dh, dh)],
                         preferred_element_type=_F32)

    row = jax.lax.broadcasted_iota(jnp.int32, (8, dh), 0)

    def ffn_gate():
        _wait_all(wg_v, wsem.at[2])
        z = jnp.dot(x_s[1].astype(_BF16), wg_v[...], preferred_element_type=_F32)
        h_s[...] = z * jax.nn.sigmoid(z)

    def ffn_up():
        _wait_all(wu_v, wsem.at[3])
        u = jnp.dot(x_s[1].astype(_BF16), wu_v[...], preferred_element_type=_F32)
        h_s[...] = h_s[...] * u

    def ffn_down():
        _wait_all(wd_v, wsem.at[4])
        bx = x_s[1]
        y = jnp.dot(h_s[...].astype(_BF16), wd_v[...], preferred_element_type=_F32)
        w_r = _as_row(wr_v)
        r = jnp.sum(bx * w_r, axis=-1, keepdims=True)
        b_s[...] = bx + (bx * 0.0 + y * jax.nn.sigmoid(r))

    side_work = (
        (2, lambda: _start_weight(wg_hbm, wg_v, wsem.at[2])),
        (5, ffn_gate),
        (6, lambda: _start_weight(wu_hbm, wu_v, wsem.at[3])),
        (9, ffn_up),
        (10, lambda: _start_weight(wd_hbm, wd_v, wsem.at[4])),
        (13, ffn_down),
    )

    def head_body(h, carry):
        for when_h, fn in side_work:
            pl.when(h == when_h)(fn)
        q = q_s[h].astype(_BF16)
        o_h = jnp.zeros((8, dh), _F32)
        for b in range(nb):
            step = h * nb + b
            slot = step % _NBUF
            more = step + _NBUF < nstep
            _wait_all(kbuf.at[slot], ksem.at[slot])
            s = jax.lax.dot_general(
                q, kbuf[slot], (((1,), (1,)), ((), ())),
                preferred_element_type=_F32) * scale
            pl.when(more)(
                functools.partial(start_cache, k_hbm, kbuf, ksem, step + _NBUF, 0))
            m = jnp.max(s, axis=-1, keepdims=True)
            e = jnp.exp(s - m)
            l = jnp.sum(e, axis=-1, keepdims=True)
            _wait_all(vbuf.at[slot], vsem.at[slot])
            o = jnp.dot(e.astype(_BF16), vbuf[slot], preferred_element_type=_F32)
            pl.when(more)(
                functools.partial(start_cache, v_hbm, vbuf, vsem, step + _NBUF, 1))
            o_h = jnp.where(row == b, o / l, o_h)
        pl.when(h == 0)(lambda: _wait_all(wo_v, wsem.at[1]))
        wo_h = wo_v[pl.ds(pl.multiple_of(h * dh, dh), dh), :]
        acc_s[...] += jnp.dot(o_h.astype(_BF16), wo_h, preferred_element_type=_F32)
        return carry

    jax.lax.fori_loop(0, nh, head_body, 0)

    g = g_s[...]
    res = g * acc_s[...] + (1.0 - g) * b_s[...]
    out_ref[...] = res[:nb].astype(out_ref.dtype)


@jax.jit
def pallas_gated_mix__mha_block_cached__moe_arch_mod__decode_kernel(
    A_x: jax.Array,
    A_k_cache: jax.Array,
    A_v_cache: jax.Array,
    A_wq: jax.Array,
    A_wo: jax.Array,
    B_x: jax.Array,
    B_w_r: jax.Array,
    B_w_gate: jax.Array,
    B_w_up: jax.Array,
    B_w_down: jax.Array,
    gate_w: jax.Array,
):
    nb, nh, sk, dh = A_k_cache.shape
    d = A_x.shape[-1]
    f = B_w_gate.shape[-1]
    ax, bx = A_x.reshape(nb, d), B_x.reshape(nb, d)
    wr, gw = B_w_r.reshape(d // 128, 128), gate_w.reshape(d // 128, 128)
    vmem = pltpu.VMEM
    scratch = [
        vmem(ax.shape, ax.dtype),
        vmem(bx.shape, bx.dtype),
        vmem(wr.shape, wr.dtype),
        vmem(gw.shape, gw.dtype),
        vmem(A_wq.shape, A_wq.dtype),
        vmem(A_wo.shape, A_wo.dtype),
        vmem(B_w_gate.shape, B_w_gate.dtype),
        vmem(B_w_up.shape, B_w_up.dtype),
        vmem(B_w_down.shape, B_w_down.dtype),
        vmem((_NBUF, sk, dh), A_k_cache.dtype),
        vmem((_NBUF, sk, dh), A_v_cache.dtype),
        vmem((2, 8, d), _F32),
        vmem((nh, 8, dh), _F32),
        vmem((8, f), _F32),
        vmem((8, d), _F32),
        vmem((8, 1), _F32),
        vmem((8, d), _F32),
        pltpu.SemaphoreType.DMA((_NBUF,)),
        pltpu.SemaphoreType.DMA((_NBUF,)),
        pltpu.SemaphoreType.DMA((5,)),
        pltpu.SemaphoreType.DMA((4,)),
    ]
    out = pl.pallas_call(
        _kernel,
        in_specs=[pl.BlockSpec(memory_space=pl.ANY)] * 11,
        out_specs=pl.BlockSpec(memory_space=pltpu.VMEM),
        out_shape=jax.ShapeDtypeStruct((nb, d), A_x.dtype),
        scratch_shapes=scratch,
        compiler_params=pltpu.CompilerParams(vmem_limit_bytes=100 * 1024 * 1024),
    )(ax, A_k_cache, A_v_cache, A_wq, A_wo, bx, wr, B_w_gate, B_w_up, B_w_down, gw)
    return out.reshape(A_x.shape)
```

```python
import functools

import jax
import jax.numpy as jnp
import jax.experimental.pallas as pl
import jax.experimental.pallas.tpu as pltpu

_NBUF = 3
_PHASES = 1
_KV_ROWS = 128
_W_ROWS = 16
_W_COLS = 1024
_F32 = jnp.float32
_BF16 = jnp.bfloat16


def _start_weight(w_hbm, w_vmem, sem):
    rows, cols = w_hbm.shape
    col_starts = list(range(0, cols, _W_COLS))
    group = 2 * _W_ROWS

    def body(i, carry):
        for half in range(2):
            r0 = pl.multiple_of(i * group + half * _W_ROWS, _W_ROWS)
            for c0 in col_starts:
                cw = min(_W_COLS, cols - c0)
                pltpu.make_async_copy(
                    w_hbm.at[pl.ds(r0, _W_ROWS), pl.ds(c0, cw)],
                    w_vmem.at[pl.ds(r0, _W_ROWS), pl.ds(c0, cw)],
                    sem,
                ).start(priority=half)
        return carry

    jax.lax.fori_loop(0, rows // group, body, 0)


def _wait_all(buf, sem):
    pltpu.make_async_copy(buf, buf, sem).wait()


def _as_row(w_ref):
    w = w_ref[...].astype(_F32)
    return jnp.concatenate([w[j:j + 1, :] for j in range(w.shape[0])], axis=1)


def _kernel(ax_hbm, k_hbm, v_hbm, wq_hbm, wo_hbm, wr_hbm, wg_hbm, wu_hbm,
            wd_hbm, gw_hbm, out_ref,
            ax_v, wr_v, gw_v, wq_v, wo_v, wg_v, wu_v, wd_v, kbuf, vbuf,
            x_s, q_s, h_s, b_s, g_s, acc_s, ksem, vsem, wsem, ssem):
    nb, nh, sk, dh = k_hbm.shape
    nstep = nb * nh
    scale = dh ** -0.5

    pieces = sk // _KV_ROWS
    per_phase = pieces // (2 * _PHASES)

    def start_kv(step, first, count):
        b = step % nb
        h = step // nb
        slot = step % _NBUF
        for j in range(first, first + count):
            rows = pl.ds(j * _KV_ROWS, _KV_ROWS)
            pltpu.make_async_copy(
                k_hbm.at[b, h, rows], kbuf.at[slot, rows], ksem.at[slot]
            ).start(priority=0)
            pltpu.make_async_copy(
                v_hbm.at[b, h, rows], vbuf.at[slot, rows], vsem.at[slot]
            ).start(priority=1)

    small = [
        pltpu.make_async_copy(ax_hbm, ax_v, ssem.at[0]),
        pltpu.make_async_copy(wr_hbm, wr_v, ssem.at[1]),
        pltpu.make_async_copy(gw_hbm, gw_v, ssem.at[2]),
    ]
    for c in small:
        c.start()
    _start_weight(wq_hbm, wq_v, wsem.at[0])

    def prologue_kv(step, carry):
        start_kv(step, 0, pieces)
        return carry

    jax.lax.fori_loop(0, _NBUF - 1, prologue_kv, 0)
    _start_weight(wo_hbm, wo_v, wsem.at[1])
    for c in small:
        c.wait()

    x_s[...] = jnp.zeros(x_s.shape, _F32)
    x_s[pl.ds(0, nb), :] = ax_v[...].astype(_F32)
    ax = x_s[...]
    gate_w = _as_row(gw_v)
    g_s[...] = jax.nn.sigmoid(jnp.sum(ax * gate_w, axis=-1, keepdims=True))
    acc_s[...] = jnp.zeros(acc_s.shape, _F32)

    _wait_all(wq_v, wsem.at[0])
    ax_bf = ax.astype(_BF16)
    for h in range(nh):
        q_s[h] = jnp.dot(ax_bf, wq_v[:, pl.ds(h * dh, dh)],
                         preferred_element_type=_F32)

    row = jax.lax.broadcasted_iota(jnp.int32, (8, dh), 0)

    def ffn_gate():
        _wait_all(wg_v, wsem.at[2])
        z = jnp.dot(x_s[...].astype(_BF16), wg_v[...], preferred_element_type=_F32)
        h_s[...] = z * jax.nn.sigmoid(z)

    def ffn_up():
        _wait_all(wu_v, wsem.at[3])
        u = jnp.dot(x_s[...].astype(_BF16), wu_v[...], preferred_element_type=_F32)
        h_s[...] = h_s[...] * u

    def ffn_down():
        _wait_all(wd_v, wsem.at[4])
        bx = x_s[...]
        y = jnp.dot(h_s[...].astype(_BF16), wd_v[...], preferred_element_type=_F32)
        w_r = _as_row(wr_v)
        r = jnp.sum(bx * w_r, axis=-1, keepdims=True)
        b_s[...] = bx + (bx * 0.0 + y * jax.nn.sigmoid(r))

    side_work = (
        (2, lambda: _start_weight(wg_hbm, wg_v, wsem.at[2])),
        (5, ffn_gate),
        (6, lambda: _start_weight(wu_hbm, wu_v, wsem.at[3])),
        (9, ffn_up),
        (10, lambda: _start_weight(wd_hbm, wd_v, wsem.at[4])),
        (13, ffn_down),
    )

    def head_body(h, carry):
        for when_h, fn in side_work:
            pl.when(h == when_h)(fn)
        q = q_s[h].astype(_BF16)
        o_h = jnp.zeros((8, dh), _F32)
        for b in range(nb):
            step = h * nb + b
            slot = step % _NBUF
            ahead = step + _NBUF - 1

            def refill(phase):
                pl.when(ahead < nstep)(functools.partial(
                    start_kv, ahead, phase * per_phase, per_phase))

            span = sk // _PHASES
            _wait_all(kbuf.at[slot], ksem.at[slot])
            s = []
            for p in range(_PHASES):
                s.append(jax.lax.dot_general(
                    q, kbuf[slot, pl.ds(p * span, span), :], (((1,), (1,)), ((), ())),
                    preferred_element_type=_F32) * scale)
                refill(p)
            s = jnp.concatenate(s, axis=1)
            m = jnp.max(s, axis=-1, keepdims=True)
            e = jnp.exp(s - m)
            l = jnp.sum(e, axis=-1, keepdims=True)
            e = e.astype(_BF16)
            _wait_all(vbuf.at[slot], vsem.at[slot])
            o = jnp.zeros((8, dh), _F32)
            for p in range(_PHASES):
                o += jnp.dot(e[:, p * span:(p + 1) * span],
                             vbuf[slot, pl.ds(p * span, span), :],
                             preferred_element_type=_F32)
                refill(_PHASES + p)
            o_h = jnp.where(row == b, o / l, o_h)
        pl.when(h == 0)(lambda: _wait_all(wo_v, wsem.at[1]))
        wo_h = wo_v[pl.ds(pl.multiple_of(h * dh, dh), dh), :]
        acc_s[...] += jnp.dot(o_h.astype(_BF16), wo_h, preferred_element_type=_F32)
        return carry

    jax.lax.fori_loop(0, nh, head_body, 0)

    g = g_s[...]
    res = g * acc_s[...] + (1.0 - g) * b_s[...]
    out_ref[...] = res[:nb].astype(out_ref.dtype)


@jax.jit
def pallas_gated_mix__mha_block_cached__moe_arch_mod__decode_kernel(
    A_x: jax.Array,
    A_k_cache: jax.Array,
    A_v_cache: jax.Array,
    A_wq: jax.Array,
    A_wo: jax.Array,
    B_x: jax.Array,
    B_w_r: jax.Array,
    B_w_gate: jax.Array,
    B_w_up: jax.Array,
    B_w_down: jax.Array,
    gate_w: jax.Array,
):
    nb, nh, sk, dh = A_k_cache.shape
    d = A_x.shape[-1]
    f = B_w_gate.shape[-1]
    del B_x
    ax = A_x.reshape(nb, d)
    wr, gw = B_w_r.reshape(d // 128, 128), gate_w.reshape(d // 128, 128)
    vmem = pltpu.VMEM
    scratch = [
        vmem(ax.shape, ax.dtype),
        vmem(wr.shape, wr.dtype),
        vmem(gw.shape, gw.dtype),
        vmem(A_wq.shape, A_wq.dtype),
        vmem(A_wo.shape, A_wo.dtype),
        vmem(B_w_gate.shape, B_w_gate.dtype),
        vmem(B_w_up.shape, B_w_up.dtype),
        vmem(B_w_down.shape, B_w_down.dtype),
        vmem((_NBUF, sk, dh), A_k_cache.dtype),
        vmem((_NBUF, sk, dh), A_v_cache.dtype),
        vmem((8, d), _F32),
        vmem((nh, 8, dh), _F32),
        vmem((8, f), _F32),
        vmem((8, d), _F32),
        vmem((8, 1), _F32),
        vmem((8, d), _F32),
        pltpu.SemaphoreType.DMA((_NBUF,)),
        pltpu.SemaphoreType.DMA((_NBUF,)),
        pltpu.SemaphoreType.DMA((5,)),
        pltpu.SemaphoreType.DMA((3,)),
    ]
    out = pl.pallas_call(
        _kernel,
        in_specs=[pl.BlockSpec(memory_space=pl.ANY)] * 10,
        out_specs=pl.BlockSpec(memory_space=pltpu.VMEM),
        out_shape=jax.ShapeDtypeStruct((nb, d), A_x.dtype),
        scratch_shapes=scratch,
        compiler_params=pltpu.CompilerParams(
            vmem_limit_bytes=100 * 1024 * 1024, disable_bounds_checks=True),
    )(ax, A_k_cache, A_v_cache, A_wq, A_wo, wr, B_w_gate, B_w_up, B_w_down, gw)
    return out.reshape(A_x.shape)
```

```python
import functools

import jax
import jax.numpy as jnp
import jax.experimental.pallas as pl
import jax.experimental.pallas.tpu as pltpu

_NBUF = 3
_KV_ROWS = 160
_KV_LEAD = 13
_W_ROWS = 16
_W_COLS = 1024
_F32 = jnp.float32
_BF16 = jnp.bfloat16


def _start_weight(w_hbm, w_vmem, sem):
    rows, cols = w_hbm.shape
    col_starts = list(range(0, cols, _W_COLS))
    group = 2 * _W_ROWS

    def body(i, carry):
        for half in range(2):
            r0 = pl.multiple_of(i * group + half * _W_ROWS, _W_ROWS)
            for c0 in col_starts:
                cw = min(_W_COLS, cols - c0)
                pltpu.make_async_copy(
                    w_hbm.at[pl.ds(r0, _W_ROWS), pl.ds(c0, cw)],
                    w_vmem.at[pl.ds(r0, _W_ROWS), pl.ds(c0, cw)],
                    sem,
                ).start(priority=half)
        return carry

    jax.lax.fori_loop(0, rows // group, body, 0)


def _kv_schedule(sk):
    pieces = [(r0, min(_KV_ROWS, sk - r0)) for r0 in range(0, sk, _KV_ROWS)]
    order = []
    for p0 in range(0, len(pieces), 2 * _KV_LEAD):
        block = pieces[p0:p0 + 2 * _KV_LEAD]
        half = (len(block) + 1) // 2
        for i in range(half):
            order.append(block[i] + (0,))
            if half + i < len(block):
                order.append(block[half + i] + (1,))
    return order


def _wait_all(buf, sem):
    pltpu.make_async_copy(buf, buf, sem).wait()


def _as_row(w_ref):
    w = w_ref[...].astype(_F32)
    return jnp.concatenate([w[j:j + 1, :] for j in range(w.shape[0])], axis=1)


def _kernel(ax_hbm, k_hbm, v_hbm, wq_hbm, wo_hbm, wr_hbm, wg_hbm, wu_hbm,
            wd_hbm, gw_hbm, out_ref,
            ax_v, wr_v, gw_v, wq_v, wo_v, wg_v, wu_v, wd_v, kbuf, vbuf,
            x_s, q_s, h_s, b_s, g_s, acc_s, ksem, vsem, wsem, ssem):
    nb, nh, sk, dh = k_hbm.shape
    nstep = nb * nh
    scale = dh ** -0.5

    def start_kv(step):
        b = step % nb
        h = step // nb
        slot = step % _NBUF
        for src, buf, sem in ((k_hbm, kbuf, ksem), (v_hbm, vbuf, vsem)):
            for r0, n, queue in _kv_schedule(sk):
                rows = pl.ds(r0, n)
                pltpu.make_async_copy(
                    src.at[b, h, rows], buf.at[slot, rows], sem.at[slot]
                ).start(priority=queue)

    small = [
        pltpu.make_async_copy(ax_hbm, ax_v, ssem.at[0]),
        pltpu.make_async_copy(wr_hbm, wr_v, ssem.at[1]),
        pltpu.make_async_copy(gw_hbm, gw_v, ssem.at[2]),
    ]
    for c in small:
        c.start()
    _start_weight(wq_hbm, wq_v, wsem.at[0])

    def prologue_kv(step, carry):
        start_kv(step)
        return carry

    jax.lax.fori_loop(0, _NBUF - 1, prologue_kv, 0)
    _start_weight(wo_hbm, wo_v, wsem.at[1])
    for c in small:
        c.wait()

    x_s[...] = jnp.zeros(x_s.shape, _F32)
    x_s[pl.ds(0, nb), :] = ax_v[...].astype(_F32)
    ax = x_s[...]
    gate_w = _as_row(gw_v)
    g_s[...] = jax.nn.sigmoid(jnp.sum(ax * gate_w, axis=-1, keepdims=True))
    acc_s[...] = jnp.zeros(acc_s.shape, _F32)

    _wait_all(wq_v, wsem.at[0])
    ax_bf = ax.astype(_BF16)
    for h in range(nh):
        q_s[h] = jnp.dot(ax_bf, wq_v[:, pl.ds(h * dh, dh)],
                         preferred_element_type=_F32)

    row = jax.lax.broadcasted_iota(jnp.int32, (8, dh), 0)

    def ffn_gate():
        _wait_all(wg_v, wsem.at[2])
        z = jnp.dot(x_s[...].astype(_BF16), wg_v[...], preferred_element_type=_F32)
        h_s[...] = z * jax.nn.sigmoid(z)

    def ffn_up():
        _wait_all(wu_v, wsem.at[3])
        u = jnp.dot(x_s[...].astype(_BF16), wu_v[...], preferred_element_type=_F32)
        h_s[...] = h_s[...] * u

    def ffn_down():
        _wait_all(wd_v, wsem.at[4])
        bx = x_s[...]
        y = jnp.dot(h_s[...].astype(_BF16), wd_v[...], preferred_element_type=_F32)
        w_r = _as_row(wr_v)
        r = jnp.sum(bx * w_r, axis=-1, keepdims=True)
        b_s[...] = bx + (bx * 0.0 + y * jax.nn.sigmoid(r))

    side_work = (
        (2, lambda: _start_weight(wg_hbm, wg_v, wsem.at[2])),
        (5, ffn_gate),
        (6, lambda: _start_weight(wu_hbm, wu_v, wsem.at[3])),
        (9, ffn_up),
        (10, lambda: _start_weight(wd_hbm, wd_v, wsem.at[4])),
        (13, ffn_down),
    )

    def head_body(h, carry):
        for when_h, fn in side_work:
            pl.when(h == when_h)(fn)
        q = q_s[h].astype(_BF16)
        o_h = jnp.zeros((8, dh), _F32)
        for b in range(nb):
            step = h * nb + b
            slot = step % _NBUF
            ahead = step + _NBUF - 1

            _wait_all(kbuf.at[slot], ksem.at[slot])
            s = jax.lax.dot_general(
                q, kbuf[slot], (((1,), (1,)), ((), ())),
                preferred_element_type=_F32) * scale
            m = jnp.max(s, axis=-1, keepdims=True)
            e = jnp.exp(s - m)
            l = jnp.sum(e, axis=-1, keepdims=True)
            _wait_all(vbuf.at[slot], vsem.at[slot])
            o = jnp.dot(e.astype(_BF16), vbuf[slot], preferred_element_type=_F32)
            pl.when(ahead < nstep)(functools.partial(start_kv, ahead))
            o_h = jnp.where(row == b, o / l, o_h)
        pl.when(h == 0)(lambda: _wait_all(wo_v, wsem.at[1]))
        wo_h = wo_v[pl.ds(pl.multiple_of(h * dh, dh), dh), :]
        acc_s[...] += jnp.dot(o_h.astype(_BF16), wo_h, preferred_element_type=_F32)
        return carry

    jax.lax.fori_loop(0, nh, head_body, 0)

    g = g_s[...]
    res = g * acc_s[...] + (1.0 - g) * b_s[...]
    out_ref[...] = res[:nb].astype(out_ref.dtype)


@jax.jit
def pallas_gated_mix__mha_block_cached__moe_arch_mod__decode_kernel(
    A_x: jax.Array,
    A_k_cache: jax.Array,
    A_v_cache: jax.Array,
    A_wq: jax.Array,
    A_wo: jax.Array,
    B_x: jax.Array,
    B_w_r: jax.Array,
    B_w_gate: jax.Array,
    B_w_up: jax.Array,
    B_w_down: jax.Array,
    gate_w: jax.Array,
):
    nb, nh, sk, dh = A_k_cache.shape
    d = A_x.shape[-1]
    f = B_w_gate.shape[-1]
    del B_x
    ax = A_x.reshape(nb, d)
    wr, gw = B_w_r.reshape(d // 128, 128), gate_w.reshape(d // 128, 128)
    vmem = pltpu.VMEM
    scratch = [
        vmem(ax.shape, ax.dtype),
        vmem(wr.shape, wr.dtype),
        vmem(gw.shape, gw.dtype),
        vmem(A_wq.shape, A_wq.dtype),
        vmem(A_wo.shape, A_wo.dtype),
        vmem(B_w_gate.shape, B_w_gate.dtype),
        vmem(B_w_up.shape, B_w_up.dtype),
        vmem(B_w_down.shape, B_w_down.dtype),
        vmem((_NBUF, sk, dh), A_k_cache.dtype),
        vmem((_NBUF, sk, dh), A_v_cache.dtype),
        vmem((8, d), _F32),
        vmem((nh, 8, dh), _F32),
        vmem((8, f), _F32),
        vmem((8, d), _F32),
        vmem((8, 1), _F32),
        vmem((8, d), _F32),
        pltpu.SemaphoreType.DMA((_NBUF,)),
        pltpu.SemaphoreType.DMA((_NBUF,)),
        pltpu.SemaphoreType.DMA((5,)),
        pltpu.SemaphoreType.DMA((3,)),
    ]
    out = pl.pallas_call(
        _kernel,
        in_specs=[pl.BlockSpec(memory_space=pl.ANY)] * 10,
        out_specs=pl.BlockSpec(memory_space=pltpu.VMEM),
        out_shape=jax.ShapeDtypeStruct((nb, d), A_x.dtype),
        scratch_shapes=scratch,
        compiler_params=pltpu.CompilerParams(
            vmem_limit_bytes=100 * 1024 * 1024, disable_bounds_checks=True),
    )(ax, A_k_cache, A_v_cache, A_wq, A_wo, wr, B_w_gate, B_w_up, B_w_down, gw)
    return out.reshape(A_x.shape)
```

```python
import functools

import jax
import jax.numpy as jnp
import jax.experimental.pallas as pl
import jax.experimental.pallas.tpu as pltpu

_NBUF = 3
_KV_ROWS = 160
_KV_LEAD = 13
_W_ROWS = 16
_W_COLS = 1024
_F32 = jnp.float32
_BF16 = jnp.bfloat16


def _start_weight(w_hbm, w_vmem, sem):
    rows, cols = w_hbm.shape
    col_starts = list(range(0, cols, _W_COLS))
    group = 2 * _W_ROWS

    def body(i, carry):
        for half in range(2):
            r0 = pl.multiple_of(i * group + half * _W_ROWS, _W_ROWS)
            for c0 in col_starts:
                cw = min(_W_COLS, cols - c0)
                pltpu.make_async_copy(
                    w_hbm.at[pl.ds(r0, _W_ROWS), pl.ds(c0, cw)],
                    w_vmem.at[pl.ds(r0, _W_ROWS), pl.ds(c0, cw)],
                    sem,
                ).start(priority=half)
        return carry

    jax.lax.fori_loop(0, rows // group, body, 0)


def _kv_schedule(sk):
    pieces = [(r0, min(_KV_ROWS, sk - r0)) for r0 in range(0, sk, _KV_ROWS)]
    order = []
    for p0 in range(0, len(pieces), 2 * _KV_LEAD):
        block = pieces[p0:p0 + 2 * _KV_LEAD]
        half = (len(block) + 1) // 2
        for i in range(half):
            order.append(block[i] + (0,))
            if half + i < len(block):
                order.append(block[half + i] + (1,))
    return order


def _wait_all(buf, sem):
    pltpu.make_async_copy(buf, buf, sem).wait()


def _as_row(w_ref):
    w = w_ref[...].astype(_F32)
    return jnp.concatenate([w[j:j + 1, :] for j in range(w.shape[0])], axis=1)


def _kernel(ax_hbm, k_hbm, v_hbm, wq_hbm, wo_hbm, wr_hbm, wg_hbm, wu_hbm,
            wd_hbm, gw_hbm, out_ref,
            ax_v, wr_v, gw_v, wq_v, wo_v, wg_v, wu_v, wd_v, kbuf, vbuf,
            x_s, h_s, b_s, g_s, acc_s, ksem, vsem, wsem, ssem):
    nb, nh, sk, dh = k_hbm.shape
    nstep = nb * nh
    scale = dh ** -0.5

    def start_kv(step):
        b = step % nb
        h = step // nb
        slot = step % _NBUF
        for src, buf, sem in ((k_hbm, kbuf, ksem), (v_hbm, vbuf, vsem)):
            for r0, n, queue in _kv_schedule(sk):
                rows = pl.ds(r0, n)
                pltpu.make_async_copy(
                    src.at[b, h, rows], buf.at[slot, rows], sem.at[slot]
                ).start(priority=queue)

    small = [
        pltpu.make_async_copy(ax_hbm, ax_v, ssem.at[0]),
        pltpu.make_async_copy(wr_hbm, wr_v, ssem.at[1]),
        pltpu.make_async_copy(gw_hbm, gw_v, ssem.at[2]),
    ]
    for c in small:
        c.start()
    _start_weight(wq_hbm, wq_v, wsem.at[0])

    def prologue_kv(step, carry):
        start_kv(step)
        return carry

    jax.lax.fori_loop(0, _NBUF - 1, prologue_kv, 0)
    _start_weight(wo_hbm, wo_v, wsem.at[1])
    for c in small:
        c.wait()

    x_s[...] = jnp.zeros(x_s.shape, _F32)
    x_s[pl.ds(0, nb), :] = ax_v[...].astype(_F32)
    ax = x_s[...]
    gate_w = _as_row(gw_v)
    g_s[...] = jax.nn.sigmoid(jnp.sum(ax * gate_w, axis=-1, keepdims=True))
    acc_s[...] = jnp.zeros(acc_s.shape, _F32)

    _wait_all(wq_v, wsem.at[0])

    row = jax.lax.broadcasted_iota(jnp.int32, (8, dh), 0)

    def ffn_gate():
        _wait_all(wg_v, wsem.at[2])
        z = jnp.dot(x_s[...].astype(_BF16), wg_v[...], preferred_element_type=_F32)
        h_s[...] = z * jax.nn.sigmoid(z)

    def ffn_up():
        _wait_all(wu_v, wsem.at[3])
        u = jnp.dot(x_s[...].astype(_BF16), wu_v[...], preferred_element_type=_F32)
        h_s[...] = h_s[...] * u

    def ffn_down():
        _wait_all(wd_v, wsem.at[4])
        bx = x_s[...]
        y = jnp.dot(h_s[...].astype(_BF16), wd_v[...], preferred_element_type=_F32)
        w_r = _as_row(wr_v)
        r = jnp.sum(bx * w_r, axis=-1, keepdims=True)
        b_s[...] = bx + (bx * 0.0 + y * jax.nn.sigmoid(r))

    side_work = (
        (2, lambda: _start_weight(wg_hbm, wg_v, wsem.at[2])),
        (5, ffn_gate),
        (6, lambda: _start_weight(wu_hbm, wu_v, wsem.at[3])),
        (9, ffn_up),
        (10, lambda: _start_weight(wd_hbm, wd_v, wsem.at[4])),
        (13, ffn_down),
    )

    def head_body(h, carry):
        for when_h, fn in side_work:
            pl.when(h == when_h)(fn)
        head = pl.ds(pl.multiple_of(h * dh, dh), dh)
        q = jnp.dot(x_s[...].astype(_BF16), wq_v[:, head],
                    preferred_element_type=_F32).astype(_BF16)
        o_h = jnp.zeros((8, dh), _F32)
        for b in range(nb):
            step = h * nb + b
            slot = step % _NBUF
            ahead = step + _NBUF - 1

            _wait_all(kbuf.at[slot], ksem.at[slot])
            s = jax.lax.dot_general(
                q, kbuf[slot], (((1,), (1,)), ((), ())),
                preferred_element_type=_F32) * scale
            m = jnp.max(s, axis=-1, keepdims=True)
            e = jnp.exp(s - m)
            l = jnp.sum(e, axis=-1, keepdims=True)
            _wait_all(vbuf.at[slot], vsem.at[slot])
            o = jnp.dot(e.astype(_BF16), vbuf[slot], preferred_element_type=_F32)
            pl.when(ahead < nstep)(functools.partial(start_kv, ahead))
            o_h = jnp.where(row == b, o / l, o_h)
        pl.when(h == 0)(lambda: _wait_all(wo_v, wsem.at[1]))
        acc_s[...] += jnp.dot(o_h.astype(_BF16), wo_v[head, :],
                              preferred_element_type=_F32)
        return carry

    jax.lax.fori_loop(0, nh, head_body, 0)

    g = g_s[...]
    res = g * acc_s[...] + (1.0 - g) * b_s[...]
    out_ref[...] = res[:nb].astype(out_ref.dtype)


@jax.jit
def pallas_gated_mix__mha_block_cached__moe_arch_mod__decode_kernel(
    A_x: jax.Array,
    A_k_cache: jax.Array,
    A_v_cache: jax.Array,
    A_wq: jax.Array,
    A_wo: jax.Array,
    B_x: jax.Array,
    B_w_r: jax.Array,
    B_w_gate: jax.Array,
    B_w_up: jax.Array,
    B_w_down: jax.Array,
    gate_w: jax.Array,
):
    nb, nh, sk, dh = A_k_cache.shape
    d = A_x.shape[-1]
    f = B_w_gate.shape[-1]
    del B_x
    ax = A_x.reshape(nb, d)
    wr, gw = B_w_r.reshape(d // 128, 128), gate_w.reshape(d // 128, 128)
    vmem = pltpu.VMEM
    scratch = [
        vmem(ax.shape, ax.dtype),
        vmem(wr.shape, wr.dtype),
        vmem(gw.shape, gw.dtype),
        vmem(A_wq.shape, A_wq.dtype),
        vmem(A_wo.shape, A_wo.dtype),
        vmem(B_w_gate.shape, B_w_gate.dtype),
        vmem(B_w_up.shape, B_w_up.dtype),
        vmem(B_w_down.shape, B_w_down.dtype),
        vmem((_NBUF, sk, dh), A_k_cache.dtype),
        vmem((_NBUF, sk, dh), A_v_cache.dtype),
        vmem((8, d), _F32),
        vmem((8, f), _F32),
        vmem((8, d), _F32),
        vmem((8, 1), _F32),
        vmem((8, d), _F32),
        pltpu.SemaphoreType.DMA((_NBUF,)),
        pltpu.SemaphoreType.DMA((_NBUF,)),
        pltpu.SemaphoreType.DMA((5,)),
        pltpu.SemaphoreType.DMA((3,)),
    ]
    out = pl.pallas_call(
        _kernel,
        in_specs=[pl.BlockSpec(memory_space=pl.ANY)] * 10,
        out_specs=pl.BlockSpec(memory_space=pltpu.VMEM),
        out_shape=jax.ShapeDtypeStruct((nb, d), A_x.dtype),
        scratch_shapes=scratch,
        compiler_params=pltpu.CompilerParams(
            vmem_limit_bytes=100 * 1024 * 1024, disable_bounds_checks=True),
    )(ax, A_k_cache, A_v_cache, A_wq, A_wo, wr, B_w_gate, B_w_up, B_w_down, gw)
    return out.reshape(A_x.shape)
```
